```python
import os as _os
_os.environ.setdefault("JAX_PLATFORMS", "cpu")
import jax
import jax.numpy as jnp

def _softmax(x, axis=-1):
    return jax.nn.softmax(x, axis=axis)
def _gelu(x):
    return jax.nn.gelu(x, approximate=True)
def _silu(x):
    return jax.nn.silu(x)
def _sigmoid(x):
    return jax.nn.sigmoid(x)
def _layernorm(x, axis=-1, eps=1e-5):
    m = jnp.mean(x, axis=axis, keepdims=True)
    v = jnp.var(x, axis=axis, keepdims=True)
    return (x - m) / jnp.sqrt(v + eps)
def _scatter_add(tgt, idx, src, axis=0):
    return tgt.at[idx].add(src)
def _segment_sum(src, seg, n):
    return jax.ops.segment_sum(src, seg, n)
class _Rng:
    def __init__(self, key):
        self._k = key
    def _next(self):
        self._k, sub = jax.random.split(self._k)
        return sub
    def normal(self, shape):
        return jax.random.normal(self._next(), shape, dtype=jnp.bfloat16)
    def randint(self, lo, hi, shape):
        return jax.random.randint(self._next(), shape, lo, hi, dtype=jnp.int32)
    def uniform(self, shape, lo=0.0, hi=1.0):
        return jax.random.uniform(self._next(), shape, jnp.bfloat16, lo, hi)
    def permutation(self, n):
        return jax.random.permutation(self._next(), n)


kernel_name = 'standalone__batchnorm__sampling'

def setup_inputs():
    _rng = _Rng(jax.random.key(int.from_bytes(__import__("os").urandom(4), "little")))
    _w = (lambda a: (lambda t: t.astype(jnp.bfloat16) if jnp.issubdtype(t.dtype, jnp.floating) else t)(jnp.asarray(a)))
    B, S, C = 1024, 8, 640
    K = 3
    return {
        "x": _w((lambda *s: _rng.normal(s) * 0.05)(B, S, C)),
        "w": _w((lambda *s: _rng.normal(s) * 0.05)(K, C, C) * (1.0 / (K * C) ** 0.5)),
        "mean": _w((lambda *s: _rng.normal(s) * 0.05)(C) * 0.1),
        "var": _w(jnp.abs((lambda *s: _rng.normal(s) * 0.05)(C)) + 0.5),
        "g": _w((lambda *s: _rng.normal(s) * 0.05)(C) + 1.0),
        "b": _w((lambda *s: _rng.normal(s) * 0.05)(C) * 0.1),
    }

def reference(x, w, mean, var, g, b):
    K = 3
    P = K // 2
    S = x.shape[1]
    xp = jnp.pad(x, ((0, 0), (P, P), (0, 0)))
    y = sum(jnp.einsum('bsc,cd->bsd', xp[:, k:k + S, :], w[k]) for k in range(K))
    inv_std = 1.0 / jnp.sqrt(var + 1e-5)
    y = (y - mean) * (g * inv_std) + b
    return _silu(y)
```

```python
import jax
import jax.numpy as jnp
from jax import lax
import jax.experimental.pallas as pl
import jax.experimental.pallas.tpu as pltpu

F32 = jnp.float32
BF16 = jnp.bfloat16
U32 = jnp.uint32

B = 1024
S = 8
C = 640
NC = C // 128
ALL = list(range(NC))
RB = NC * S
RU = RB // 2
CH = 8

A = 1.5
A2 = A * A
SS = A2 + 1.0 / A2
NA = 2.0 * (A2 * A2 - 1.0)
NB = -NA / (A2 * A2)

BE = 256
S1, S2 = 128, 256
SP = S1 + S2
NIT = 2
XL0 = BE + S1
assert BE + NIT * SP == B


def _t(b0, b1, cs, g=32, kind='t'):
    return [(kind, b, c, g) for b in range(b0, b1, g) for c in cs]


def _t2(cs, kind='t'):
    return _t(0, 32, cs, 16, kind) + _t(32, 96, cs, 32, kind)


def _x(b0, b1):
    return [('x', b, k) for b in range(b0, b1, CH) for k in range(NC)]


def _w(c):
    return [('w', c, r) for r in range(C // 16)]


XP = [(0, 32), (32, 96), (96, 128), (128, 192), (192, 384)]
VP = [(0, 16), (16, 32), (32, 64), (64, 96), (96, 128), (128, 192), (192, 256)]
OP = [(0, 128), (128, 256)]
LXP = [(XL0, 512), (512, 768), (768, 1024)]
LOP = [(0, 128), (128, 256), (256, 320), (320, 352), (352, 368), (368, 384)]
STARTS = ['w0', 'p', 'x0', 'x1', 'w1', 'w2', 'x2', 'w3', 'w4', 'x3', 'x4', 'l0', 'l1', 'l2']

SEGS = [
    (['w0', 'p'], [], [], ['pp'] + _w(0), 0),
    (['x0'], [], [], _x(0, 16), 0),
    ([], [], _t(0, 16, [0], 16), _x(16, 32), 'D'),
    ([], [], _t(16, 32, [0], 16), [], 0),
    (['x1'], [], [], _x(32, 64), 0),
    ([], [], _t(32, 64, [0]), _x(64, 96), 'D'),
    ([], [], _t(64, 96, [0]), [], 0),
    (['w1'], [], _t2([1], 'r'), _w(1), 'D'),
    ([], [], _t2([1], 'f'), [], 0),
    (['w2', 'x2'], [], _t2([2], 'r'), _w(2), 'D'),
    ([], [], _t2([2], 'f'), _x(96, 128), 4),
    ([], [], _t(96, 128, [0, 1, 2]), [], 0),
    (['w3', 'w4', 'x3'], [], _t2([3], 'r'), _w(3), 'D'),
    ([], [], _t2([3], 'f') + _t(96, 128, [3]), _w(4), 6),
    ([], [], _t2([4]) + _t(96, 128, [4]), _x(128, 192), (5, 128)),
    (['x4'], [], _t(128, 192, ALL), _x(192, 288), 0),
    ([], [], _t(192, 256, ALL), _x(288, 384), (14, 256)),
]
LSEGS = [
    ([], [], _t(0, S1, ALL), _x(S1, SP), 8),
    ([], [0], _t(S1, 256, ALL), _x(SP, SP + S1), 0),
    ([], [1], _t(256, 320, ALL), [], (0, SP)),
    ([], [2], _t(320, 352, ALL), [], 0),
    ([], [3], _t(352, 368, ALL, 16), [], 0),
    ([], [4], _t(368, 384, ALL, 16), [], 0),
    ([], [5], [], [], 0),
]
_DOTS = {'t': (0, 1, 2, 3, 4, 5), 'r': (0, 5), 'f': (1, 2, 3, 4)}


def _piece(pieces, b):
    for n, (b0, b1) in enumerate(pieces):
        if b0 <= b < b1:
            return n, b - b0
    raise ValueError(b)


def _unpack(u):
    lo = lax.bitcast_convert_type(u << 16, F32)
    hi = lax.bitcast_convert_type(u & jnp.uint32(0xFFFF0000), F32)
    return lo, hi


def _pack(lo, hi):
    lo = lax.bitcast_convert_type(lo.astype(BF16).astype(F32), U32)
    hi = lax.bitcast_convert_type(hi.astype(BF16).astype(F32), U32)
    return (lo >> 16) | hi


def _in_tf(d0, d1, d2, d3, d4, d5):
    v0 = d4 - SS * d2
    if d0 is not None:
        v0 = v0 + d0
    v5 = d1 - SS * d3
    if d5 is not None:
        v5 = v5 + d5
    e1 = d4 - (1.0 / A2) * d2
    o1 = A * d3 - (1.0 / A) * d1
    e2 = d4 - A2 * d2
    o2 = (1.0 / A) * d3 - A * d1
    return v0, e1 + o1, e1 - o1, e2 + o2, e2 - o2, v5


def _kernel(zero_ref, x_hbm, w_hbm, mean_hbm, var_hbm, g_hbm, b_hbm, o_hbm, *scr):
    scr = list(scr)

    def take(n):
        return [scr.pop(0) for _ in range(n)]

    xb = take(len(XP))
    (xl,) = take(1)
    vb = take(len(VP))
    va_ref, vb_ref = take(2)
    ob = take(len(OP))
    lob = take(len(LOP))
    wb = take(NC)
    ub = take(NC)
    qs = take(4)
    p_ref, pace, isem, osem = scr
    zero = zero_ref[0]
    zvec = jnp.zeros((8, 128), U32)

    def l_copy(n, b0, nb):
        return pltpu.make_async_copy(x_hbm.at[pl.ds(b0 * RB, nb * RB)],
                                     xl.at[pl.ds((b0 - XL0) * RB, nb * RB)],
                                     isem.at[4 + NC + len(XP) + n])

    def lo_copy(it, j):
        r0, r1 = LOP[j]
        row = pl.multiple_of((BE + it * SP + r0) * RB, 16)
        return pltpu.make_async_copy(lob[j].at[it], o_hbm.at[pl.ds(row, (r1 - r0) * RB)],
                                     osem.at[len(OP) + it * len(LOP) + j])

    def copies(name):
        kind = name[0]
        if kind == 'p':
            return [pltpu.make_async_copy(s, d, isem.at[i]) for i, (s, d) in
                    enumerate(zip((mean_hbm, var_hbm, g_hbm, b_hbm), qs))]
        n = int(name[1:])
        if kind == 'w':
            return [pltpu.make_async_copy(w_hbm.at[:, :, pl.ds(n * 128, 128)], wb[n], isem.at[4 + n])]
        if kind == 'x':
            b0, b1 = XP[n]
            return [pltpu.make_async_copy(x_hbm.at[pl.ds(b0 * RB, (b1 - b0) * RB)], xb[n],
                                          isem.at[4 + NC + n])]
        if kind == 'l':
            b0, b1 = LXP[n]
            return [l_copy(n, b0, b1 - b0)]
        b0, b1 = OP[n]
        return [pltpu.make_async_copy(ob[n], o_hbm.at[pl.ds(b0 * RB, (b1 - b0) * RB)], osem.at[n])]

    def wait0(nm):
        for cp in copies(nm):
            cp.wait()

    def start0(nm):
        for cp in copies(nm):
            cp.start()

    for nm in STARTS:
        start0(nm)

    wu = [r.bitcast(U32) for r in wb]
    uu = [r.bitcast(U32) for r in ub]
    u_st = [r.at[pl.ds(zero, 5)] for r in ub]
    pace_st = pace.at[pl.ds(zero, 2)]
    pace[1] = zvec
    for r in uu:
        r[4, 0:8, :] = zvec
    for r in vb + [va_ref, vb_ref]:
        r.bitcast(U32)[6, 0, 0:8, :] = zvec

    def params():
        mean, var, g, b = [q[...].astype(F32).reshape(1, C) for q in qs]
        scale = (0.5 * g) * lax.rsqrt(var + 1e-5)
        shift = 0.5 * b - mean * scale
        p_ref[0] = jnp.broadcast_to(scale, (8, C))
        p_ref[1] = jnp.broadcast_to(shift, (8, C))

    def w_chunk(c, r, tok):
        sc = p_ref[0, 0:1, c * 128:(c + 1) * 128]
        ws = [wu[c][t, r * 8:(r + 1) * 8, :] for t in range(3)]
        if tok is not None:
            ws = [w_ | tok for w_ in ws]
        g0, g1, g2 = [pltpu.bitcast(w_, BF16).astype(F32) for w_ in ws]
        ea = (g0 + A2 * g2) * (sc * (1.0 / NA))
        oa = g1 * (sc * (A / NA))
        eb = (g0 + (1.0 / A2) * g2) * (sc * (1.0 / NB))
        ob_ = g1 * (sc * (1.0 / (A * NB)))
        rs = slice(r * 16, (r + 1) * 16)
        u_st[c][0, rs, :] = (ea + oa).astype(BF16)
        u_st[c][1, rs, :] = (ea - oa).astype(BF16)
        u_st[c][2, rs, :] = (eb + ob_).astype(BF16)
        u_st[c][3, rs, :] = (eb - ob_).astype(BF16)

    def run(segs, xmap, vmap, omap, do_wait, do_start):
        state = {'m': None}
        held = {}

        def in_chunk(b, k, tok):
            xr, b0 = xmap(b)
            xs = []
            for j in range(4):
                u = xr[pl.ds(b0 * RU + k * 4 + j, CH, stride=RU), :]
                if tok is not None:
                    u = u | tok
                xs += list(_unpack(u))
            va = _in_tf(None, xs[0], xs[1], xs[2], xs[3], xs[4])
            vb_ = _in_tf(xs[3], xs[4], xs[5], xs[6], xs[7], None)
            vr, bv = vmap(b)
            vst = vr.at[pl.ds(zero, 7)]
            for i in range(6):
                vst[i, k, 2 * bv:2 * bv + 16, :] = jnp.concatenate([va[i], vb_[i]], axis=0).astype(BF16)

        def side_op(s_, tok):
            if s_ == 'pp':
                params()
            elif s_[0] == 'x':
                in_chunk(s_[1], s_[2], tok)
            else:
                w_chunk(s_[1], s_[2], tok)

        def v_token(b):
            return vmap(b)[0].bitcast(U32)[6, 0, 0:8, :]

        def task(kind, b, c, g, pre, post):
            vr, bv = vmap(b)
            vru = vr.bitcast(U32)
            m = held.pop((b, c), [None] * 6)
            for i in _DOTS[kind]:
                parts = [vru[i, k, bv:bv + g, :] for k in range(NC)]
                tok = pre()
                if tok is not None:
                    parts[0] = jnp.concatenate([parts[0][0:8] | tok, parts[0][8:]], axis=0)
                lhs = pltpu.bitcast(jnp.concatenate(parts, axis=1), BF16)
                rhs = wu[c][0] if i == 0 else wu[c][2] if i == 5 else uu[c][i - 1]
                m[i] = jnp.dot(lhs, pltpu.bitcast(rhs, BF16), preferred_element_type=F32)
                state['m'] = m[i]
                post()
            if kind == 'r':
                held[(b, c)] = m
                return
            sc = p_ref[0, 0:1, c * 128:(c + 1) * 128]
            sh = p_ref[1, 0:1, c * 128:(c + 1) * 128]
            s1 = m[1] + m[2]
            t1 = m[1] - m[2]
            s2 = m[3] + m[4]
            t2 = m[3] - m[4]
            h0 = (sc * m[0] + sh) + (s1 + s2)
            h1 = (A * t1 + sh) + (1.0 / A) * t2
            h2 = (A2 * s1 + sh) + (1.0 / A2) * s2
            h3 = (A2 * A * t1 + sh) + ((1.0 / (A2 * A)) * t2 + sc * m[5])
            ys = [h * jnp.tanh(h) + h for h in (h0, h1, h2, h3)]
            ps = (_pack(ys[0], ys[1]), _pack(ys[2], ys[3]))
            orf, bo = omap(b)
            for h in range(2):
                for q in range(2 * g // 8):
                    base = (bo + (q // 2) * 8) * RU + c * 4 + 2 * (q % 2) + h
                    orf[pl.ds(base, 8, stride=RU), :] = ps[h][q * 8:(q + 1) * 8]

        def segment(main, side, mode):
            npts = sum(len(_DOTS[t[0]]) for t in main)
            st = {'pt': 0, 'done': 0}

            if mode == 'D':
                def pre_d():
                    d = st['pt']
                    st['pt'] += 1
                    if d == 0:
                        return None
                    upto = int(round(len(side) * d / npts))
                    for s_ in side[st['done']:upto]:
                        side_op(s_, None)
                    st['done'] = upto
                    return uu[side[0][1]][4, 0:8, :] if side[0][0] == 'w' else v_token(side[0][1])

                for t in main:
                    task(*t, pre_d, lambda: None)
                for s_ in side[st['done']:]:
                    side_op(s_, None)
                return

            margin, fake = mode if isinstance(mode, tuple) else (mode, None)
            last = max(npts - margin, 1)

            def emit():
                upto = min(len(side), -(-(st['pt'] + 1) * len(side) // last))
                todo = side[st['done']:upto]
                for idx, s_ in enumerate(todo):
                    tok = None
                    mi = state['m']
                    if mi is not None:
                        r0 = (idx * (mi.shape[0] // 8) // len(todo)) * 8
                        pace_st[0] = lax.bitcast_convert_type(mi[r0:r0 + 8], U32)
                        tok = pace[1]
                    side_op(s_, tok)
                st['done'] = upto
                st['pt'] += 1

            def pre():
                if fake is not None and st['pt'] == npts:
                    return v_token(fake)
                return None

            emit()
            for t in main:
                task(*t, pre, emit)
            assert st['done'] == len(side)

        for waits, starts, main, side, mode in segs:
            if waits:
                for nm in waits:
                    do_wait(nm)
                state['m'] = None
            for nm in starts:
                do_start(nm)
            segment(main, side, mode)
        assert not held

    xu = [r.bitcast(U32) for r in xb]
    ou = [r.bitcast(U32) for r in ob]

    def xmap0(b):
        n, b0 = _piece(XP, b)
        return xu[n], b0

    def vmap0(b):
        if b >= BE:
            return va_ref, b - BE
        n, b0 = _piece(VP, b)
        return vb[n], b0

    def omap0(b):
        n, b0 = _piece(OP, b)
        return ou[n], b0

    run(SEGS, xmap0, vmap0, omap0, wait0, start0)
    wait0('l0')
    start0('o0')
    start0('o1')

    def body(it, carry):
        l_copy(1 + it, pl.multiple_of(512 + it * 256, 16), 256).wait()
        r1 = pl.multiple_of(it * (SP * RB), 16)
        r2 = pl.multiple_of(jnp.minimum(it * SP + S2, B - XL0 - S1) * RB, 16)
        x1 = xl.at[pl.ds(r1, S2 * RB)].bitcast(U32)
        x2 = xl.at[pl.ds(r2, S1 * RB)].bitcast(U32)
        lou = [r.at[it].bitcast(U32) for r in lob]

        def xmap(b):
            return (x1, b - S1) if b < SP else (x2, b - SP)

        def vmap(b):
            if b < S1:
                return va_ref, b
            if b < SP:
                return vb_ref, b - S1
            return va_ref, b - SP

        def omap(b):
            n, b0 = _piece(LOP, b)
            return lou[n], b0

        run(LSEGS, xmap, vmap, omap, None, lambda j: lo_copy(it, j).start())
        for j in range(len(LOP) - 1):
            lo_copy(it, j).wait()
        return carry

    lax.fori_loop(0, NIT, body, 0)

    for n in range(len(OP)):
        wait0('o%d' % n)
    for it in range(NIT):
        lo_copy(it, len(LOP) - 1).wait()


@jax.jit
def pallas_standalone__batchnorm__sampling_kernel(
    x: jax.Array,
    w: jax.Array,
    mean: jax.Array,
    var: jax.Array,
    g: jax.Array,
    b: jax.Array,
):
    assert x.shape == (B, S, C) and w.shape == (3, C, C)
    z = x.reshape(B, S, NC, 128).transpose(0, 2, 1, 3).reshape(B * RB, 128)
    anyspec = pl.BlockSpec(memory_space=pl.ANY)

    def rows(nb):
        return pltpu.VMEM((nb * RB, 128), BF16)

    def vbuf(nb):
        return pltpu.VMEM((7, NC, 2 * nb, 128), BF16)

    scratch = ([rows(b1 - b0) for b0, b1 in XP]
               + [rows(B - XL0)]
               + [vbuf(b1 - b0) for b0, b1 in VP]
               + [vbuf(S1), vbuf(S2)]
               + [rows(b1 - b0) for b0, b1 in OP]
               + [pltpu.VMEM((NIT, (b1 - b0) * RB, 128), BF16) for b0, b1 in LOP]
               + [pltpu.VMEM((3, C, 128), BF16) for _ in range(NC)]
               + [pltpu.VMEM((5, C, 128), BF16) for _ in range(NC)]
               + [pltpu.VMEM((C,), BF16) for _ in range(4)]
               + [pltpu.VMEM((2, 8, C), F32),
                  pltpu.VMEM((2, 8, 128), U32),
                  pltpu.SemaphoreType.DMA((4 + NC + len(XP) + len(LXP),)),
                  pltpu.SemaphoreType.DMA((len(OP) + NIT * len(LOP),))])
    out = pl.pallas_call(
        _kernel,
        grid_spec=pltpu.PrefetchScalarGridSpec(
            num_scalar_prefetch=1,
            grid=(1,),
            in_specs=[anyspec] * 6,
            out_specs=anyspec,
            scratch_shapes=scratch),
        out_shape=jax.ShapeDtypeStruct(z.shape, x.dtype),
        compiler_params=pltpu.CompilerParams(
            dimension_semantics=("arbitrary",),
            vmem_limit_bytes=100 * 1024 * 1024,
            disable_bounds_checks=True,
            disable_semaphore_checks=True),
    )(jnp.zeros((1,), jnp.int32), z, w, mean, var, g, b)
    return out.reshape(B, NC, S, 128).transpose(0, 2, 1, 3).reshape(B, S, C)
```

```python
import jax
import jax.numpy as jnp
from jax import lax
import jax.experimental.pallas as pl
import jax.experimental.pallas.tpu as pltpu

F32 = jnp.float32
BF16 = jnp.bfloat16
U32 = jnp.uint32

B = 1024
S = 8
C = 640
NC = C // 128
ALL = list(range(NC))
RB = NC * S
RU = RB // 2
CH = 16
NP = 11

KS = 512.5 / 90.0
KD = 511.5 / 150.0
KAP = KS - 4.0 / 9.0

BE = 192
S1, S2 = 160, 256
SP = S1 + S2
NIT = 2
XL0 = BE + S1
assert BE + NIT * SP == B


def _t(b0, b1, cs, g=64, kind='t'):
    return [(kind, b, c, g) for b in range(b0, b1, g) for c in cs]


def _t3(cs, kind):
    return _t(32, 96, cs, 64, kind) + _t(0, 32, cs, 32, kind)


def _x(b0, b1):
    return [('x', b, k) for b in range(b0, b1, CH) for k in range(NC)]


def _w(c, which='ab'):
    return [('w', c, r, which) for r in range(C // 16)]


XP = [(0, 32), (32, 96), (96, 128), (128, 192), (192, 352)]
VP = [(0, 32), (32, 64), (64, 96), (96, 128), (128, 192)]
OP = [(0, 128), (128, 192)]
LXP = [(XL0, XL0 + S2), (XL0 + S2, B)]
LOP = [(0, 160), (160, 288), (288, 352), (352, 384), (384, 416)]
STARTS = ['w0', 'p', 'x0', 'x1', 'w1', 'w2', 'x2', 'w3', 'w4', 'x3', 'x4', 'l0', 'l1']

SEGS = [
    (['w0', 'p'], [], [], ['pp'] + _w(0), 0),
    (['x0'], [], [], _x(0, 32), 0),
    ([], [], _t(0, 32, [0], 32), [], 0),
    (['x1'], [], [], _x(32, 64), 0),
    ([], [], _t(32, 64, [0], 32), _x(64, 96), 'D'),
    ([], [], _t(64, 96, [0], 32), [], 0),
    (['w1'], [], _t3([1], 'r'), _w(1, 'a'), ('E', 1, 2)),
    ([], [], _t3([1], 'a'), _w(1, 'b'), ('E', 0, 2)),
    ([], [], _t3([1], 'b'), [], 0),
    (['w2', 'x2'], [], _t3([2], 'r'), _w(2, 'a'), ('E', 1, 2)),
    ([], [], _t3([2], 'a'), _x(96, 128), ('E', 0, 1)),
    ([], [], _t(96, 128, [0], 32), _w(2, 'b'), ('E', 0, 8)),
    ([], [], _t3([2], 'b'), [], 0),
    ([], [], _t(96, 128, [1, 2], 32), [], 0),
    (['w3', 'w4', 'x3'], [], _t(0, 128, [3], 64, 'r') + _t(0, 128, [4], 64, 'r'), _w(3), ('E', 1, 2)),
    ([], [], _t(0, 128, [3], 64, 'a'), _w(4)[:30], ('E', 0, 0)),
    ([], [], _t(0, 128, [3], 64, 'b'), _w(4)[30:] + _x(128, 144), ('E', 0, 20)),
    ([], [], _t(0, 128, [4], 64, 'a'), _x(144, 192), ('E', 6, 0)),
    ([], [], _t(0, 128, [4], 64, 'b'), [], 0),
    (['x4'], [], _t(128, 192, [0, 1, 2, 3]) + _t(128, 192, [4], 32), _x(192, 352), ('A', 26, 192)),
]
LSEGS = [
    ([], [], _t(0, 128, ALL) + _t(128, S1, ALL, 32), _x(S1, SP), ('A', 40, S1)),
    (['mid'], [0], _t(S1, 288, ALL), _x(SP, SP + S1), 0),
    ([], [1], _t(288, 352, ALL), [], 0),
    ([], [2], _t(352, 384, ALL, 32), [], 0),
    ([], [3], _t(384, 416, ALL, 32), [], ('A', 0, SP)),
    ([], [4], [], [], 0),
]
_DOTS = {'t': (2, 3, 4, 5, 6, 7, 8, 0, 9, 1, 10),
         'r': (2, 0, 1), 'a': (3, 4, 5, 6), 'b': (7, 8, 9, 10)}


def _piece(pieces, b):
    for n, (b0, b1) in enumerate(pieces):
        if b0 <= b < b1:
            return n, b - b0
    raise ValueError(b)


def _unpack(u):
    lo = lax.bitcast_convert_type(u << 16, F32)
    hi = lax.bitcast_convert_type(u & jnp.uint32(0xFFFF0000), F32)
    return lo, hi


def _pack(lo, hi):
    lo = lax.bitcast_convert_type(lo.astype(BF16).astype(F32), U32)
    hi = lax.bitcast_convert_type(hi.astype(BF16).astype(F32), U32)
    return (lo >> 16) | hi


def _horner(a, b, c, d):
    return ((0.25 * a + b) * 0.25 + c) * 0.25 + d


def _in_tf(x):
    p, q = x[0] + x[4], x[2] + x[6]
    e1, ei = p + q, p - q
    p, q = x[1] + x[5], x[3] + x[7]
    o1, oi = p + q, p - q
    e2 = 0.5 * _horner(x[0], x[2], x[4], x[6])
    o2 = _horner(x[1], x[3], x[5], x[7])
    eh = 2.0 * _horner(x[6], x[4], x[2], x[0])
    oh = _horner(x[7], x[5], x[3], x[1])
    return (x[0], x[7], ei + oi, e1 + o1, e1 - o1, e2 + o2, e2 - o2, eh + oh, eh - oh, ei, oi)


def _out_tf(m, sc2, sh):
    k1 = sc2 * m[2]
    k16 = 0.16 * k1
    s1, t1 = m[3] + m[4], m[3] - m[4]
    a, t2 = m[5] + m[6], m[5] - m[6]
    b, th4 = m[7] + m[8], 0.25 * (m[7] - m[8])
    sh2 = sh + sh
    out = [None] * 8
    for r1, pp, mm, kk, c, ml, sg, off in ((s1, a + b, a - b, 256.0, m[0], m[9], 1.0, 1),
                                           (t1, t2 + th4, t2 - th4, 512.0, m[1], m[10], -1.0, 0)):
        u1 = (kk / 90.0) * pp - ((4.0 / 9.0) * r1 - sh)
        u2 = (r1 + sh2) - u1
        v1 = (kk / 150.0) * mm - k16
        v2 = v1 + k1
        c = sc2 * c
        u1 = u1 - KAP * c
        u2 = u2 + (KAP - 1.0) * c
        v1 = v1 + (sg * (KD - 0.16)) * c
        v2 = v2 + (sg * (KD + 0.84)) * c
        v1 = v1 + (sg * 0.32) * ml
        v2 = v2 - (sg * 1.68) * ml
        out[off + 0] = u1 - v1
        out[off + 2] = u2 - v2
        out[off + 4] = u2 + v2
        out[off + 6] = u1 + v1
    return out


def _kernel(zero_ref, x_hbm, w_hbm, mean_hbm, var_hbm, g_hbm, b_hbm, o_hbm, *scr):
    scr = list(scr)

    def take(n):
        return [scr.pop(0) for _ in range(n)]

    xb = take(len(XP))
    (xl,) = take(1)
    vb = take(len(VP))
    va_ref, vb_ref = take(2)
    ob = take(len(OP))
    lob = take(len(LOP))
    wb = take(NC)
    ua = take(NC)
    ub = take(NC)
    qs = take(4)
    p_ref, pace, isem, osem = scr
    zero = zero_ref[0]
    zvec = jnp.zeros((8, 128), U32)

    def lo_copy(it, j):
        r0, r1 = LOP[j]
        row = pl.multiple_of((BE + it * SP + r0) * RB, 16)
        return pltpu.make_async_copy(lob[j].at[it], o_hbm.at[pl.ds(row, (r1 - r0) * RB)],
                                     osem.at[len(OP) + it * len(LOP) + j])

    def copies(name):
        kind = name[0]
        if kind == 'p':
            return [pltpu.make_async_copy(s, d, isem.at[i]) for i, (s, d) in
                    enumerate(zip((mean_hbm, var_hbm, g_hbm, b_hbm), qs))]
        n = int(name[1:])
        if kind == 'w':
            return [pltpu.make_async_copy(w_hbm.at[:, :, pl.ds(n * 128, 128)], wb[n], isem.at[4 + n])]
        if kind == 'x':
            b0, b1 = XP[n]
            return [pltpu.make_async_copy(x_hbm.at[pl.ds(b0 * RB, (b1 - b0) * RB)], xb[n],
                                          isem.at[4 + NC + n])]
        if kind == 'l':
            b0, b1 = LXP[n]
            return [pltpu.make_async_copy(x_hbm.at[pl.ds(b0 * RB, (b1 - b0) * RB)],
                                          xl.at[pl.ds((b0 - XL0) * RB, (b1 - b0) * RB)],
                                          isem.at[4 + NC + len(XP) + n])]
        b0, b1 = OP[n]
        return [pltpu.make_async_copy(ob[n], o_hbm.at[pl.ds(b0 * RB, (b1 - b0) * RB)], osem.at[n])]

    def wait0(nm):
        for cp in copies(nm):
            cp.wait()

    def start0(nm):
        for cp in copies(nm):
            cp.start()

    for nm in STARTS:
        start0(nm)

    wu = [r.bitcast(U32) for r in wb]
    uau = [r.bitcast(U32) for r in ua]
    ubu = [r.bitcast(U32) for r in ub]
    ua_st = [r.at[pl.ds(zero, 5)] for r in ua]
    ub_st = [r.at[pl.ds(zero, 5)] for r in ub]
    pace_st = pace.at[pl.ds(zero, 2)]
    pace[1] = zvec
    for r in uau + ubu:
        r[4, 0:8, :] = zvec
    for r in vb + [va_ref, vb_ref]:
        r.bitcast(U32)[NP, 0, 0:8, :] = zvec

    def params():
        mean, var, g, b = [q[...].astype(F32).reshape(1, C) for q in qs]
        scale = (0.5 * g) * lax.rsqrt(var + 1e-5)
        shift = 0.5 * b - mean * scale
        p_ref[0] = jnp.broadcast_to(0.5 * scale, (8, C))
        p_ref[1] = jnp.broadcast_to(shift, (8, C))
        p_ref[2] = jnp.broadcast_to(0.25 * scale, (8, C))

    def w_chunk(c, r, which, tok):
        sc4 = p_ref[2, 0:1, c * 128:(c + 1) * 128]
        ws = [wu[c][t, r * 8:(r + 1) * 8, :] for t in range(3)]
        if tok is not None:
            ws = [w_ | tok for w_ in ws]
        g0, g1, g2 = [pltpu.bitcast(w_, BF16).astype(F32) * sc4 for w_ in ws]
        gh = 0.5 * g1
        rs = slice(r * 16, (r + 1) * 16)
        if 'a' in which:
            for n, (e, o) in enumerate(((g0 + g2, g1), (0.25 * g2 + g0, gh))):
                ua_st[c][2 * n, rs, :] = (e + o).astype(BF16)
                ua_st[c][2 * n + 1, rs, :] = (e - o).astype(BF16)
        if 'b' in which:
            for n, (e, o) in enumerate(((0.25 * g0 + g2, gh), (g2 - g0, g1))):
                ub_st[c][2 * n, rs, :] = (e + o).astype(BF16)
                ub_st[c][2 * n + 1, rs, :] = (e - o).astype(BF16)

    def rhs_of(c, i):
        if i < 3:
            return wu[c][(2, 0, 1)[i]]
        return uau[c][i - 3] if i < 7 else ubu[c][i - 7]

    def run(segs, xmap, vmap, omap, do_wait, do_start):
        state = {'m': None, 'prod': 0}
        held = {}

        def in_chunk(b, k, tok):
            xr, b0 = xmap(b)
            xs = []
            for j in range(4):
                u = xr[pl.ds(b0 * RU + k * 4 + j, CH, stride=RU), :]
                if tok is not None:
                    u = u | jnp.concatenate([tok] * (CH // 8), axis=0)
                xs += list(_unpack(u))
            v = _in_tf(xs)
            vr, bv = vmap(b)
            vst = vr.at[pl.ds(zero, NP + 1)]
            for i in range(NP):
                vst[i, k, bv:bv + CH, :] = v[i].astype(BF16)

        def side_op(s_, tok):
            if s_ == 'pp':
                params()
            elif s_[0] == 'x':
                in_chunk(s_[1], s_[2], tok)
            else:
                w_chunk(s_[1], s_[2], s_[3], tok)

        def v_token(b):
            return vmap(b)[0].bitcast(U32)[NP, 0, 0:8, :]

        def done_token(todo):
            srcs = {}
            for s_ in todo:
                if s_[0] == 'x':
                    srcs[('x', id(vmap(s_[1])[0]))] = lambda b=s_[1]: v_token(b)
                else:
                    for ch, us in (('a', uau), ('b', ubu)):
                        if ch in s_[3]:
                            srcs[(ch, s_[1])] = lambda r=us[s_[1]]: r[4, 0:8, :]
            tok = None
            for f in srcs.values():
                tok = f() if tok is None else tok | f()
            return tok

        def task(kind, b, c, g, pre, fine, post):
            spans = []
            for bb in range(b, b + g, 32):
                vr, bv = vmap(bb)
                if spans and spans[-1][0] is vr:
                    spans[-1][2] += 32
                else:
                    spans.append([vr, bv, 32])
            spans = [(vr.bitcast(U32), bv, n) for vr, bv, n in spans]
            m = held.pop((b, c), [None] * NP)
            for i in _DOTS[kind]:
                parts = [jnp.concatenate([vru[i, k, bv // 2:(bv + n) // 2, :] for vru, bv, n in spans], axis=0)
                         for k in range(NC)]
                tok = pre()
                if tok is not None:
                    parts[0] = jnp.concatenate([parts[0][0:8] | tok, parts[0][8:]], axis=0)
                for k in range(NC):
                    if fine is not None and state['prod'] % 4 == 0:
                        rows = []
                        for q in range(g // 16):
                            tok = fine()
                            r_ = parts[k][q * 8:(q + 1) * 8]
                            rows.append(r_ if tok is None else r_ | tok)
                        parts[k] = jnp.concatenate(rows, axis=0)
                    state['prod'] += 1
                lhs = pltpu.bitcast(jnp.concatenate(parts, axis=1), BF16)
                m[i] = jnp.dot(lhs, pltpu.bitcast(rhs_of(c, i), BF16), preferred_element_type=F32)
                state['m'] = m[i]
                post()
            if kind in 'ra':
                held[(b, c)] = m
                return
            sc2 = p_ref[0, 0:1, c * 128:(c + 1) * 128]
            sh = p_ref[1, 0:1, c * 128:(c + 1) * 128]
            ys = [h * jnp.tanh(h) + h for h in _out_tf(m, sc2, sh)]
            for j in range(4):
                pk = _pack(ys[2 * j], ys[2 * j + 1])
                for q in range(g // 8):
                    orf, bo = omap(b + q * 8)
                    orf[pl.ds(bo * RU + c * 4 + j, 8, stride=RU), :] = pk[q * 8:(q + 1) * 8]

        def nothing():
            return None

        def segment(main, side, mode):
            npts = sum(len(_DOTS[t[0]]) for t in main)
            st = {'pt': 0, 'done': 0}

            def advance(upto):
                todo = side[st['done']:upto]
                for s_ in todo:
                    side_op(s_, None)
                st['done'] = max(st['done'], upto)
                return done_token(todo)

            if mode == 'D' or (isinstance(mode, tuple) and mode[0] == 'E'):
                if mode == 'D':
                    skip, use = 1, npts
                else:
                    p_, tot = state['prod'], 0
                    for t in main:
                        for _ in range(len(_DOTS[t[0]]) * NC):
                            tot += t[3] // 16 if p_ % 4 == 0 else 0
                            p_ += 1
                    skip, use = mode[1], max(tot - mode[1] - mode[2], 1)

                def point():
                    d = st['pt'] - skip + 1
                    st['pt'] += 1
                    return advance(min(len(side), int(round(len(side) * d / use))) if d > 0 else 0)

                for t in main:
                    if mode == 'D':
                        task(*t, point, None, nothing)
                    else:
                        task(*t, nothing, point, nothing)
                for s_ in side[st['done']:]:
                    side_op(s_, None)
                return

            margin, fake = mode[1:] if isinstance(mode, tuple) else (mode, None)
            last = max(npts - margin, 1)

            def emit():
                upto = min(len(side), -(-(st['pt'] + 1) * len(side) // last))
                todo = side[st['done']:upto]
                for idx, s_ in enumerate(todo):
                    tok = None
                    mi = state['m']
                    if mi is not None:
                        r0 = (idx * (mi.shape[0] // 8) // len(todo)) * 8
                        pace_st[0] = lax.bitcast_convert_type(mi[r0:r0 + 8], U32)
                        tok = pace[1]
                    side_op(s_, tok)
                st['done'] = upto
                st['pt'] += 1

            def pre():
                if fake is not None and st['pt'] == npts:
                    return v_token(fake)
                return None

            emit()
            for t in main:
                task(*t, pre, None, emit)
            assert st['done'] == len(side)

        for waits, starts, main, side, mode in segs:
            if waits:
                for nm in waits:
                    do_wait(nm)
                state['m'] = None
                state['prod'] = 0
            for nm in starts:
                do_start(nm)
            segment(main, side, mode)
        assert not held

    xu = [r.bitcast(U32) for r in xb]
    ou = [r.bitcast(U32) for r in ob]

    def xmap0(b):
        n, b0 = _piece(XP, b)
        return xu[n], b0

    def vmap0(b):
        if b >= BE:
            return va_ref, b - BE
        n, b0 = _piece(VP, b)
        return vb[n], b0

    def omap0(b):
        n, b0 = _piece(OP, b)
        return ou[n], b0

    run(SEGS, xmap0, vmap0, omap0, wait0, start0)
    wait0('l0')

    def body(it, carry):
        r1 = pl.multiple_of(it * (SP * RB), 16)
        r2 = pl.multiple_of(jnp.minimum(it * SP + S2, B - XL0 - S1) * RB, 16)
        x1 = xl.at[pl.ds(r1, S2 * RB)].bitcast(U32)
        x2 = xl.at[pl.ds(r2, S1 * RB)].bitcast(U32)
        lou = [r.at[it].bitcast(U32) for r in lob]

        def mid(_):
            @pl.when(it == 0)
            def _():
                wait0('l1')
                start0('o0')
                start0('o1')

        def xmap(b):
            return (x1, b - S1) if b < SP else (x2, b - SP)

        def vmap(b):
            if b < S1:
                return va_ref, b
            if b < SP:
                return vb_ref, b - S1
            return va_ref, b - SP

        def omap(b):
            n, b0 = _piece(LOP, b)
            return lou[n], b0

        run(LSEGS, xmap, vmap, omap, mid, lambda j: lo_copy(it, j).start())
        for j in range(len(LOP) - 1):
            lo_copy(it, j).wait()
        return carry

    lax.fori_loop(0, NIT, body, 0)

    for n in range(len(OP)):
        wait0('o%d' % n)
    for it in range(NIT):
        lo_copy(it, len(LOP) - 1).wait()


@jax.jit
def pallas_standalone__batchnorm__sampling_kernel(
    x: jax.Array,
    w: jax.Array,
    mean: jax.Array,
    var: jax.Array,
    g: jax.Array,
    b: jax.Array,
):
    assert x.shape == (B, S, C) and w.shape == (3, C, C)
    z = x.reshape(B, S, NC, 128).transpose(0, 2, 1, 3).reshape(B * RB, 128)
    anyspec = pl.BlockSpec(memory_space=pl.ANY)

    def rows(nb):
        return pltpu.VMEM((nb * RB, 128), BF16)

    def vbuf(nb):
        return pltpu.VMEM((NP + 1, NC, nb, 128), BF16)

    scratch = ([rows(b1 - b0) for b0, b1 in XP]
               + [rows(B - XL0)]
               + [vbuf(b1 - b0) for b0, b1 in VP]
               + [vbuf(S1), vbuf(S2)]
               + [rows(b1 - b0) for b0, b1 in OP]
               + [pltpu.VMEM((NIT, (b1 - b0) * RB, 128), BF16) for b0, b1 in LOP]
               + [pltpu.VMEM((3, C, 128), BF16) for _ in range(NC)]
               + [pltpu.VMEM((5, C, 128), BF16) for _ in range(2 * NC)]
               + [pltpu.VMEM((C,), BF16) for _ in range(4)]
               + [pltpu.VMEM((3, 8, C), F32),
                  pltpu.VMEM((2, 8, 128), U32),
                  pltpu.SemaphoreType.DMA((4 + NC + len(XP) + len(LXP),)),
                  pltpu.SemaphoreType.DMA((len(OP) + NIT * len(LOP),))])
    out = pl.pallas_call(
        _kernel,
        grid_spec=pltpu.PrefetchScalarGridSpec(
            num_scalar_prefetch=1,
            grid=(1,),
            in_specs=[anyspec] * 6,
            out_specs=anyspec,
            scratch_shapes=scratch),
        out_shape=jax.ShapeDtypeStruct(z.shape, x.dtype),
        compiler_params=pltpu.CompilerParams(
            dimension_semantics=("arbitrary",),
            vmem_limit_bytes=100 * 1024 * 1024,
            disable_bounds_checks=True,
            disable_semaphore_checks=True),
    )(jnp.zeros((1,), jnp.int32), z, w, mean, var, g, b)
    return out.reshape(B, NC, S, 128).transpose(0, 2, 1, 3).reshape(B, S, C)
```

```python
import jax
import jax.numpy as jnp
from jax import lax
import jax.experimental.pallas as pl
import jax.experimental.pallas.tpu as pltpu

F32 = jnp.float32
BF16 = jnp.bfloat16
U32 = jnp.uint32

B = 1024
S = 8
C = 640
NC = C // 128
ALL = list(range(NC))
RB = NC * S
RU = RB // 2
CH = 16
NP = 11

KS = 512.5 / 90.0
KD = 511.5 / 150.0
KAP = KS - 4.0 / 9.0

BE = 192
S1, S2 = 160, 256
SP = S1 + S2
NIT = 2
XL0 = BE + S1
assert BE + NIT * SP == B


def _t(b0, b1, cs, g=64, kind='t'):
    return [(kind, b, c, g) for b in range(b0, b1, g) for c in cs]


def _t3(cs, kind):
    return _t(32, 96, cs, 64, kind) + _t(0, 32, cs, 32, kind)


def _x(b0, b1):
    return [('x', b, k) for b in range(b0, b1, CH) for k in range(NC)]


def _w(c, which='ab'):
    return [('w', c, r, which) for r in range(C // 16)]


XP = [(0, 32), (32, 96), (96, 128), (128, 192), (192, 352)]
VP = [(0, 32), (32, 64), (64, 96), (96, 128), (128, 192)]
OP = [(0, 128), (128, 192)]
LXP = [(XL0, XL0 + S2), (XL0 + S2, B)]
LOP = [(0, 160), (160, 288), (288, 352), (352, 384), (384, 416)]
STARTS = ['w0', 'p', 'x0', 'x1', 'w1', 'w2', 'x2', 'w3', 'w4', 'x3', 'x4', 'l0', 'l1']

SEGS = [
    (['w0', 'p'], [], [], ['pp'] + _w(0), 0),
    (['x0'], [], [], _x(0, 32), 0),
    ([], [], _t(0, 32, [0], 32), [], 0),
    (['x1'], [], [], _x(32, 64), 0),
    ([], [], _t(32, 64, [0], 32), _x(64, 96), 'D'),
    ([], [], _t(64, 96, [0], 32), [], 0),
    (['w1'], [], _t3([1], 'r'), _w(1, 'a'), ('E', 1, 2)),
    ([], [], _t3([1], 'a'), _w(1, 'b'), ('E', 0, 2)),
    ([], [], _t3([1], 'b'), [], 0),
    (['w2', 'x2'], [], _t3([2], 'r'), _w(2, 'a'), ('E', 1, 2)),
    ([], [], _t3([2], 'a'), _x(96, 128), ('E', 0, 1)),
    ([], [], _t(96, 128, [0], 32), _w(2, 'b'), ('E', 0, 8)),
    ([], [], _t3([2], 'b'), [], 0),
    ([], [], _t(96, 128, [1, 2], 32), [], 0),
    (['w3', 'w4', 'x3'], [], _t(0, 128, [3], 64, 'r') + _t(0, 128, [4], 64, 'r'), _w(3), ('E', 1, 2)),
    ([], [], _t(0, 128, [3], 64, 'a'), _w(4)[:30], ('E', 0, 0)),
    ([], [], _t(0, 128, [3], 64, 'b'), _w(4)[30:] + _x(128, 144), ('E', 0, 20)),
    ([], [], _t(0, 128, [4], 64, 'a'), _x(144, 192), ('E', 6, 0)),
    ([], [], _t(0, 128, [4], 64, 'b'), [], 0),
    (['x4'], [], _t(128, 192, [0, 1, 2, 3]) + _t(128, 192, [4], 32), _x(192, 352), ('A', 26, 192)),
]
LSEGS = [
    ([], [], _t(0, 128, ALL) + _t(128, S1, ALL, 32), _x(S1, SP), ('A', 40, S1)),
    (['mid'], [], _t(S1, 288, ALL), _x(SP, SP + S1), 0),
    ([], [1], _t(288, 352, ALL), [], 0),
    ([], [2], _t(352, 384, ALL, 32), [], 0),
    ([], [3], _t(384, 416, ALL, 32), [], ('A', 0, SP)),
    ([], [4], [], [], 0),
]
_DOTS = {'t': (2, 3, 4, 5, 6, 7, 8, 0, 9, 1, 10),
         'r': (2, 0, 1), 'a': (3, 4, 5, 6), 'b': (7, 8, 9, 10)}


def _piece(pieces, b):
    for n, (b0, b1) in enumerate(pieces):
        if b0 <= b < b1:
            return n, b - b0
    raise ValueError(b)


def _unpack(u):
    lo = lax.bitcast_convert_type(u << 16, F32)
    hi = lax.bitcast_convert_type(u & jnp.uint32(0xFFFF0000), F32)
    return lo, hi


def _pack(lo, hi):
    lo = lax.bitcast_convert_type(lo.astype(BF16).astype(F32), U32)
    hi = lax.bitcast_convert_type(hi.astype(BF16).astype(F32), U32)
    return (lo >> 16) | hi


def _horner(a, b, c, d):
    return ((0.25 * a + b) * 0.25 + c) * 0.25 + d


def _in_tf(x):
    p, q = x[0] + x[4], x[2] + x[6]
    e1, ei = p + q, p - q
    p, q = x[1] + x[5], x[3] + x[7]
    o1, oi = p + q, p - q
    e2 = 0.5 * _horner(x[0], x[2], x[4], x[6])
    o2 = _horner(x[1], x[3], x[5], x[7])
    eh = 2.0 * _horner(x[6], x[4], x[2], x[0])
    oh = _horner(x[7], x[5], x[3], x[1])
    return (x[0], x[7], ei + oi, e1 + o1, e1 - o1, e2 + o2, e2 - o2, eh + oh, eh - oh, ei, oi)


def _out_tf(m, sc2, sh):
    k1 = sc2 * m[2]
    k16 = 0.16 * k1
    s1, t1 = m[3] + m[4], m[3] - m[4]
    a, t2 = m[5] + m[6], m[5] - m[6]
    b, th4 = m[7] + m[8], 0.25 * (m[7] - m[8])
    sh2 = sh + sh
    out = [None] * 8
    for r1, pp, mm, kk, c, ml, sg, off in ((s1, a + b, a - b, 256.0, m[0], m[9], 1.0, 1),
                                           (t1, t2 + th4, t2 - th4, 512.0, m[1], m[10], -1.0, 0)):
        u1 = (kk / 90.0) * pp - ((4.0 / 9.0) * r1 - sh)
        u2 = (r1 + sh2) - u1
        v1 = (kk / 150.0) * mm - k16
        v2 = v1 + k1
        c = sc2 * c
        u1 = u1 - KAP * c
        u2 = u2 + (KAP - 1.0) * c
        v1 = v1 + (sg * (KD - 0.16)) * c
        v2 = v2 + (sg * (KD + 0.84)) * c
        v1 = v1 + (sg * 0.32) * ml
        v2 = v2 - (sg * 1.68) * ml
        out[off + 0] = u1 - v1
        out[off + 2] = u2 - v2
        out[off + 4] = u2 + v2
        out[off + 6] = u1 + v1
    return out


def _kernel(zero_ref, x_hbm, w_hbm, mean_hbm, var_hbm, g_hbm, b_hbm, o_hbm, *scr):
    scr = list(scr)

    def take(n):
        return [scr.pop(0) for _ in range(n)]

    xb = take(len(XP))
    (xl,) = take(1)
    vb = take(len(VP))
    va_ref, vb_ref = take(2)
    ob = take(len(OP))
    lob = take(len(LOP))
    wb = take(NC)
    ua = take(NC)
    ub = take(NC)
    qs = take(4)
    p_ref, pace, isem, osem = scr
    zero = zero_ref[0]
    zvec = jnp.zeros((8, 128), U32)

    def lo_copy(it, j):
        r0, r1 = LOP[j]
        row = pl.multiple_of((BE + it * SP + r0) * RB, 16)
        return pltpu.make_async_copy(lob[j].at[it], o_hbm.at[pl.ds(row, (r1 - r0) * RB)],
                                     osem.at[len(OP) + it * len(LOP) + j])

    def copies(name):
        kind = name[0]
        if kind == 'p':
            return [pltpu.make_async_copy(s, d, isem.at[i]) for i, (s, d) in
                    enumerate(zip((mean_hbm, var_hbm, g_hbm, b_hbm), qs))]
        n = int(name[1:])
        if kind == 'w':
            return [pltpu.make_async_copy(w_hbm.at[:, :, pl.ds(n * 128, 128)], wb[n], isem.at[4 + n])]
        if kind == 'x':
            b0, b1 = XP[n]
            return [pltpu.make_async_copy(x_hbm.at[pl.ds(b0 * RB, (b1 - b0) * RB)], xb[n],
                                          isem.at[4 + NC + n])]
        if kind == 'l':
            b0, b1 = LXP[n]
            return [pltpu.make_async_copy(x_hbm.at[pl.ds(b0 * RB, (b1 - b0) * RB)],
                                          xl.at[pl.ds((b0 - XL0) * RB, (b1 - b0) * RB)],
                                          isem.at[4 + NC + len(XP) + n])]
        b0, b1 = OP[n]
        return [pltpu.make_async_copy(ob[n], o_hbm.at[pl.ds(b0 * RB, (b1 - b0) * RB)], osem.at[n])]

    def wait0(nm):
        for cp in copies(nm):
            cp.wait()

    def start0(nm):
        for cp in copies(nm):
            cp.start()

    for nm in STARTS:
        start0(nm)

    wu = [r.bitcast(U32) for r in wb]
    uau = [r.bitcast(U32) for r in ua]
    ubu = [r.bitcast(U32) for r in ub]
    ua_st = [r.at[pl.ds(zero, 5)] for r in ua]
    ub_st = [r.at[pl.ds(zero, 5)] for r in ub]
    pace_st = pace.at[pl.ds(zero, 2)]
    pace[1] = zvec
    for r in uau + ubu:
        r[4, 0:8, :] = zvec
    for r in vb + [va_ref, vb_ref]:
        r.bitcast(U32)[NP, 0, 0:8, :] = zvec

    def params():
        mean, var, g, b = [q[...].astype(F32).reshape(1, C) for q in qs]
        scale = (0.5 * g) * lax.rsqrt(var + 1e-5)
        shift = 0.5 * b - mean * scale
        p_ref[0] = jnp.broadcast_to(0.5 * scale, (8, C))
        p_ref[1] = jnp.broadcast_to(shift, (8, C))
        p_ref[2] = jnp.broadcast_to(0.25 * scale, (8, C))

    def w_chunk(c, r, which, tok):
        sc4 = p_ref[2, 0:1, c * 128:(c + 1) * 128]
        ws = [wu[c][t, r * 8:(r + 1) * 8, :] for t in range(3)]
        if tok is not None:
            ws = [w_ | tok for w_ in ws]
        g0, g1, g2 = [pltpu.bitcast(w_, BF16).astype(F32) * sc4 for w_ in ws]
        gh = 0.5 * g1
        rs = slice(r * 16, (r + 1) * 16)
        if 'a' in which:
            for n, (e, o) in enumerate(((g0 + g2, g1), (0.25 * g2 + g0, gh))):
                ua_st[c][2 * n, rs, :] = (e + o).astype(BF16)
                ua_st[c][2 * n + 1, rs, :] = (e - o).astype(BF16)
        if 'b' in which:
            for n, (e, o) in enumerate(((0.25 * g0 + g2, gh), (g2 - g0, g1))):
                ub_st[c][2 * n, rs, :] = (e + o).astype(BF16)
                ub_st[c][2 * n + 1, rs, :] = (e - o).astype(BF16)

    def rhs_of(c, i):
        if i < 3:
            return wu[c][(2, 0, 1)[i]]
        return uau[c][i - 3] if i < 7 else ubu[c][i - 7]

    def run(segs, xmap, vmap, omap, do_wait, do_start):
        state = {'m': None, 'prod': 0}
        held = {}

        def in_chunk(b, k, tok):
            xr, b0 = xmap(b)
            xs = []
            for j in range(4):
                u = xr[pl.ds(b0 * RU + k * 4 + j, CH, stride=RU), :]
                if tok is not None:
                    u = u | jnp.concatenate([tok] * (CH // 8), axis=0)
                xs += list(_unpack(u))
            v = _in_tf(xs)
            vr, bv = vmap(b)
            vst = vr.at[pl.ds(zero, NP + 1)]
            for i in range(NP):
                vst[i, k, bv:bv + CH, :] = v[i].astype(BF16)

        def side_op(s_, tok):
            if s_ == 'pp':
                params()
            elif s_[0] == 'x':
                in_chunk(s_[1], s_[2], tok)
            else:
                w_chunk(s_[1], s_[2], s_[3], tok)

        def v_token(b):
            return vmap(b)[0].bitcast(U32)[NP, 0, 0:8, :]

        def done_token(todo):
            srcs = {}
            for s_ in todo:
                if s_[0] == 'x':
                    srcs[('x', id(vmap(s_[1])[0]))] = lambda b=s_[1]: v_token(b)
                else:
                    for ch, us in (('a', uau), ('b', ubu)):
                        if ch in s_[3]:
                            srcs[(ch, s_[1])] = lambda r=us[s_[1]]: r[4, 0:8, :]
            tok = None
            for f in srcs.values():
                tok = f() if tok is None else tok | f()
            return tok

        def task(kind, b, c, g, pre, fine, post):
            spans = []
            for bb in range(b, b + g, 32):
                vr, bv = vmap(bb)
                if spans and spans[-1][0] is vr:
                    spans[-1][2] += 32
                else:
                    spans.append([vr, bv, 32])
            spans = [(vr.bitcast(U32), bv, n) for vr, bv, n in spans]
            m = held.pop((b, c), [None] * NP)
            for i in _DOTS[kind]:
                parts = [jnp.concatenate([vru[i, k, bv // 2:(bv + n) // 2, :] for vru, bv, n in spans], axis=0)
                         for k in range(NC)]
                tok = pre()
                if tok is not None:
                    parts[0] = jnp.concatenate([parts[0][0:8] | tok, parts[0][8:]], axis=0)
                for k in range(NC):
                    if fine is not None and state['prod'] % 4 == 0:
                        rows = []
                        for q in range(g // 16):
                            tok = fine()
                            r_ = parts[k][q * 8:(q + 1) * 8]
                            rows.append(r_ if tok is None else r_ | tok)
                        parts[k] = jnp.concatenate(rows, axis=0)
                    state['prod'] += 1
                lhs = pltpu.bitcast(jnp.concatenate(parts, axis=1), BF16)
                m[i] = jnp.dot(lhs, pltpu.bitcast(rhs_of(c, i), BF16), preferred_element_type=F32)
                state['m'] = m[i]
                post()
            if kind in 'ra':
                held[(b, c)] = m
                return
            sc2 = p_ref[0, 0:1, c * 128:(c + 1) * 128]
            sh = p_ref[1, 0:1, c * 128:(c + 1) * 128]
            ys = [h * jnp.tanh(h) + h for h in _out_tf(m, sc2, sh)]
            for j in range(4):
                pk = _pack(ys[2 * j], ys[2 * j + 1])
                for q in range(g // 8):
                    orf, bo = omap(b + q * 8)
                    orf[pl.ds(bo * RU + c * 4 + j, 8, stride=RU), :] = pk[q * 8:(q + 1) * 8]

        def nothing():
            return None

        def segment(main, side, mode):
            npts = sum(len(_DOTS[t[0]]) for t in main)
            st = {'pt': 0, 'done': 0}

            def advance(upto):
                todo = side[st['done']:upto]
                for s_ in todo:
                    side_op(s_, None)
                st['done'] = max(st['done'], upto)
                return done_token(todo)

            if mode == 'D' or (isinstance(mode, tuple) and mode[0] == 'E'):
                if mode == 'D':
                    skip, use = 1, npts
                else:
                    p_, tot = state['prod'], 0
                    for t in main:
                        for _ in range(len(_DOTS[t[0]]) * NC):
                            tot += t[3] // 16 if p_ % 4 == 0 else 0
                            p_ += 1
                    skip, use = mode[1], max(tot - mode[1] - mode[2], 1)

                def point():
                    d = st['pt'] - skip + 1
                    st['pt'] += 1
                    return advance(min(len(side), int(round(len(side) * d / use))) if d > 0 else 0)

                for t in main:
                    if mode == 'D':
                        task(*t, point, None, nothing)
                    else:
                        task(*t, nothing, point, nothing)
                for s_ in side[st['done']:]:
                    side_op(s_, None)
                return

            margin, fake = mode[1:] if isinstance(mode, tuple) else (mode, None)
            last = max(npts - margin, 1)

            def emit():
                upto = min(len(side), -(-(st['pt'] + 1) * len(side) // last))
                todo = side[st['done']:upto]
                for idx, s_ in enumerate(todo):
                    tok = None
                    mi = state['m']
                    if mi is not None:
                        r0 = (idx * (mi.shape[0] // 8) // len(todo)) * 8
                        pace_st[0] = lax.bitcast_convert_type(mi[r0:r0 + 8], U32)
                        tok = pace[1]
                    side_op(s_, tok)
                st['done'] = upto
                st['pt'] += 1

            def pre():
                if fake is not None and st['pt'] == npts:
                    return v_token(fake)
                return None

            emit()
            for t in main:
                task(*t, pre, None, emit)
            assert st['done'] == len(side)

        for waits, starts, main, side, mode in segs:
            if waits:
                for nm in waits:
                    do_wait(nm)
                state['m'] = None
                state['prod'] = 0
            for nm in starts:
                do_start(nm)
            segment(main, side, mode)
        assert not held

    xu = [r.bitcast(U32) for r in xb]
    ou = [r.bitcast(U32) for r in ob]

    def xmap0(b):
        n, b0 = _piece(XP, b)
        return xu[n], b0

    def vmap0(b):
        if b >= BE:
            return va_ref, b - BE
        n, b0 = _piece(VP, b)
        return vb[n], b0

    def omap0(b):
        n, b0 = _piece(OP, b)
        return ou[n], b0

    run(SEGS, xmap0, vmap0, omap0, wait0, start0)
    wait0('l0')

    def body(it, carry):
        r1 = pl.multiple_of(it * (SP * RB), 16)
        r2 = pl.multiple_of(jnp.minimum(it * SP + S2, B - XL0 - S1) * RB, 16)
        x1 = xl.at[pl.ds(r1, S2 * RB)].bitcast(U32)
        x2 = xl.at[pl.ds(r2, S1 * RB)].bitcast(U32)
        lou = [r.at[it].bitcast(U32) for r in lob]

        def mid(_):
            lo_copy(it, 0).start()

            @pl.when(it == 0)
            def _():
                start0('o0')
                start0('o1')
                wait0('l1')

        def xmap(b):
            return (x1, b - S1) if b < SP else (x2, b - SP)

        def vmap(b):
            if b < S1:
                return va_ref, b
            if b < SP:
                return vb_ref, b - S1
            return va_ref, b - SP

        def omap(b):
            n, b0 = _piece(LOP, b)
            return lou[n], b0

        run(LSEGS, xmap, vmap, omap, mid, lambda j: lo_copy(it, j).start())
        for j in range(len(LOP) - 1):
            lo_copy(it, j).wait()
        return carry

    lax.fori_loop(0, NIT, body, 0)

    for n in range(len(OP)):
        wait0('o%d' % n)
    for it in range(NIT):
        lo_copy(it, len(LOP) - 1).wait()


def _compiler_params():
    kw = dict(dimension_semantics=("arbitrary",),
              vmem_limit_bytes=100 * 1024 * 1024,
              disable_bounds_checks=True)
    try:
        return pltpu.CompilerParams(disable_semaphore_checks=True, **kw)
    except TypeError:
        return pltpu.CompilerParams(**kw)


@jax.jit
def pallas_standalone__batchnorm__sampling_kernel(
    x: jax.Array,
    w: jax.Array,
    mean: jax.Array,
    var: jax.Array,
    g: jax.Array,
    b: jax.Array,
):
    assert x.shape == (B, S, C) and w.shape == (3, C, C)
    z = x.reshape(B, S, NC, 128).transpose(0, 2, 1, 3).reshape(B * RB, 128)
    anyspec = pl.BlockSpec(memory_space=pl.ANY)

    def rows(nb):
        return pltpu.VMEM((nb * RB, 128), BF16)

    def vbuf(nb):
        return pltpu.VMEM((NP + 1, NC, nb, 128), BF16)

    scratch = ([rows(b1 - b0) for b0, b1 in XP]
               + [rows(B - XL0)]
               + [vbuf(b1 - b0) for b0, b1 in VP]
               + [vbuf(S1), vbuf(S2)]
               + [rows(b1 - b0) for b0, b1 in OP]
               + [pltpu.VMEM((NIT, (b1 - b0) * RB, 128), BF16) for b0, b1 in LOP]
               + [pltpu.VMEM((3, C, 128), BF16) for _ in range(NC)]
               + [pltpu.VMEM((5, C, 128), BF16) for _ in range(2 * NC)]
               + [pltpu.VMEM((C,), BF16) for _ in range(4)]
               + [pltpu.VMEM((3, 8, C), F32),
                  pltpu.VMEM((2, 8, 128), U32),
                  pltpu.SemaphoreType.DMA((4 + NC + len(XP) + len(LXP),)),
                  pltpu.SemaphoreType.DMA((len(OP) + NIT * len(LOP),))])
    out = pl.pallas_call(
        _kernel,
        grid_spec=pltpu.PrefetchScalarGridSpec(
            num_scalar_prefetch=1,
            grid=(1,),
            in_specs=[anyspec] * 6,
            out_specs=anyspec,
            scratch_shapes=scratch),
        out_shape=jax.ShapeDtypeStruct(z.shape, x.dtype),
        compiler_params=_compiler_params(),
    )(jnp.zeros((1,), jnp.int32), z, w, mean, var, g, b)
    return out.reshape(B, NC, S, 128).transpose(0, 2, 1, 3).reshape(B, S, C)
```

```python
import jax
import jax.numpy as jnp
from jax import lax
import jax.experimental.pallas as pl
import jax.experimental.pallas.tpu as pltpu

F32 = jnp.float32
BF16 = jnp.bfloat16
U32 = jnp.uint32

B = 1024
S = 8
C = 640
NC = C // 128
ALL = list(range(NC))
RB = NC * S
RU = RB // 2
CH = 16
NP = 11

KS = 512.5 / 90.0
KD = 511.5 / 150.0
KAP = KS - 4.0 / 9.0

BE = 192
S1, S2 = 160, 256
SP = S1 + S2
NIT = 2
XL0 = BE + S1
assert BE + NIT * SP == B


def _t(b0, b1, cs, g=64, kind='t'):
    return [(kind, b, c, g) for b in range(b0, b1, g) for c in cs]


def _t3(cs, kind):
    return _t(32, 96, cs, 64, kind) + _t(0, 32, cs, 32, kind)


def _x(b0, b1):
    return [('x', b, k) for b in range(b0, b1, CH) for k in range(NC)]


def _w(c, which='ab'):
    return [('w', c, r, which) for r in range(C // 16)]


XP = [(0, 32), (32, 96), (96, 128), (128, 192), (192, 352)]
VP = [(0, 32), (32, 64), (64, 96), (96, 128), (128, 192)]
OP = [(0, 128), (128, 192)]
LXP = [(XL0, XL0 + S2), (XL0 + S2, B)]
LOP = [(0, 160), (160, 288), (288, 352), (352, 384), (384, 416)]
STARTS = ['w0', 'p', 'x0', 'x1', 'w1', 'w2', 'x2', 'w3', 'w4', 'x3', 'x4', 'l0', 'l1']

SEGS = [
    (['w0', 'p'], [], [], ['pp'] + _w(0), 0),
    (['x0'], [], [], _x(0, 32), 0),
    ([], [], _t(0, 32, [0], 32), [], 0),
    (['x1'], [], [], _x(32, 64), 0),
    ([], [], _t(32, 64, [0], 32), _x(64, 96), 'D'),
    ([], [], _t(64, 96, [0], 32), [], 0),
    (['w1'], [], _t3([1], 'r'), _w(1, 'a'), ('E', 1, 2)),
    ([], [], _t3([1], 'a'), _w(1, 'b'), ('E', 0, 2)),
    ([], [], _t3([1], 'b'), [], 0),
    (['w2', 'x2'], [], _t3([2], 'r'), _w(2, 'a'), ('E', 1, 2)),
    ([], [], _t3([2], 'a'), _w(2, 'b'), ('E', 0, 2)),
    ([], [], _t3([2], 'b'), _x(96, 128), ('E', 0, 8)),
    (['w3'], [], _t(96, 128, [0, 1, 2], 32), _w(3), ('E', 1, 4)),
    (['w4', 'x3'], [], _t(0, 128, [4], 64, 'r') + _t(0, 64, [3]), _w(4), ('E', 1, 30)),
    ([], [], _t(64, 128, [3]) + _t(0, 128, [4], 64, 'a'), _x(128, 192), 5),
    ([], [], _t(0, 128, [4], 64, 'b'), [], ('A', 0, 128)),
    (['x4'], [], _t(128, 192, [0, 1, 2, 3]) + _t(128, 192, [4], 32), _x(192, 352), ('A', 26, 192)),
]
LSEGS = [
    ([], [], _t(0, 128, ALL) + _t(128, S1, ALL, 32), _x(S1, SP), ('A', 40, S1)),
    (['mid'], [], _t(S1, 288, ALL), _x(SP, SP + S1), 0),
    ([], [1], _t(288, 352, ALL), [], 0),
    ([], [2], _t(352, 384, ALL, 32), [], 0),
    ([], [3], _t(384, 416, ALL, 32), [], ('A', 0, SP)),
    ([], [4], [], [], 0),
]
_DOTS = {'t': (2, 3, 4, 5, 6, 7, 8, 0, 9, 1, 10),
         'r': (2, 0, 1), 'a': (3, 4, 5, 6), 'b': (7, 8, 9, 10)}


def _piece(pieces, b):
    for n, (b0, b1) in enumerate(pieces):
        if b0 <= b < b1:
            return n, b - b0
    raise ValueError(b)


def _unpack(u):
    lo = lax.bitcast_convert_type(u << 16, F32)
    hi = lax.bitcast_convert_type(u & jnp.uint32(0xFFFF0000), F32)
    return lo, hi


def _pack(lo, hi):
    lo = lax.bitcast_convert_type(lo.astype(BF16).astype(F32), U32)
    hi = lax.bitcast_convert_type(hi.astype(BF16).astype(F32), U32)
    return (lo >> 16) | hi


def _horner(a, b, c, d):
    return ((0.25 * a + b) * 0.25 + c) * 0.25 + d


def _in_tf(x):
    p, q = x[0] + x[4], x[2] + x[6]
    e1, ei = p + q, p - q
    p, q = x[1] + x[5], x[3] + x[7]
    o1, oi = p + q, p - q
    e2 = 0.5 * _horner(x[0], x[2], x[4], x[6])
    o2 = _horner(x[1], x[3], x[5], x[7])
    eh = 2.0 * _horner(x[6], x[4], x[2], x[0])
    oh = _horner(x[7], x[5], x[3], x[1])
    return (x[0], x[7], ei + oi, e1 + o1, e1 - o1, e2 + o2, e2 - o2, eh + oh, eh - oh, ei, oi)


def _out_tf(m, sc2, sh):
    k1 = sc2 * m[2]
    k16 = 0.16 * k1
    s1, t1 = m[3] + m[4], m[3] - m[4]
    a, t2 = m[5] + m[6], m[5] - m[6]
    b, th4 = m[7] + m[8], 0.25 * (m[7] - m[8])
    sh2 = sh + sh
    out = [None] * 8
    for r1, pp, mm, kk, c, ml, sg, off in ((s1, a + b, a - b, 256.0, m[0], m[9], 1.0, 1),
                                           (t1, t2 + th4, t2 - th4, 512.0, m[1], m[10], -1.0, 0)):
        u1 = (kk / 90.0) * pp - ((4.0 / 9.0) * r1 - sh)
        u2 = (r1 + sh2) - u1
        v1 = (kk / 150.0) * mm - k16
        v2 = v1 + k1
        c = sc2 * c
        u1 = u1 - KAP * c
        u2 = u2 + (KAP - 1.0) * c
        v1 = v1 + (sg * (KD - 0.16)) * c
        v2 = v2 + (sg * (KD + 0.84)) * c
        v1 = v1 + (sg * 0.32) * ml
        v2 = v2 - (sg * 1.68) * ml
        out[off + 0] = u1 - v1
        out[off + 2] = u2 - v2
        out[off + 4] = u2 + v2
        out[off + 6] = u1 + v1
    return out


def _kernel(zero_ref, x_hbm, w_hbm, mean_hbm, var_hbm, g_hbm, b_hbm, o_hbm, *scr):
    scr = list(scr)

    def take(n):
        return [scr.pop(0) for _ in range(n)]

    xb = take(len(XP))
    (xl,) = take(1)
    vb = take(len(VP))
    va_ref, vb_ref = take(2)
    ob = take(len(OP))
    lob = take(len(LOP))
    wb = take(NC)
    ua = take(NC)
    ub = take(NC)
    qs = take(4)
    p_ref, pace, isem, osem = scr
    zero = zero_ref[0]
    zvec = jnp.zeros((8, 128), U32)

    def lo_copy(it, j):
        r0, r1 = LOP[j]
        row = pl.multiple_of((BE + it * SP + r0) * RB, 16)
        return pltpu.make_async_copy(lob[j].at[it], o_hbm.at[pl.ds(row, (r1 - r0) * RB)],
                                     osem.at[len(OP) + it * len(LOP) + j])

    def copies(name):
        kind = name[0]
        if kind == 'p':
            return [pltpu.make_async_copy(s, d, isem.at[i]) for i, (s, d) in
                    enumerate(zip((mean_hbm, var_hbm, g_hbm, b_hbm), qs))]
        n = int(name[1:])
        if kind == 'w':
            return [pltpu.make_async_copy(w_hbm.at[:, :, pl.ds(n * 128, 128)], wb[n], isem.at[4 + n])]
        if kind == 'x':
            b0, b1 = XP[n]
            return [pltpu.make_async_copy(x_hbm.at[pl.ds(b0 * RB, (b1 - b0) * RB)], xb[n],
                                          isem.at[4 + NC + n])]
        if kind == 'l':
            b0, b1 = LXP[n]
            return [pltpu.make_async_copy(x_hbm.at[pl.ds(b0 * RB, (b1 - b0) * RB)],
                                          xl.at[pl.ds((b0 - XL0) * RB, (b1 - b0) * RB)],
                                          isem.at[4 + NC + len(XP) + n])]
        b0, b1 = OP[n]
        return [pltpu.make_async_copy(ob[n], o_hbm.at[pl.ds(b0 * RB, (b1 - b0) * RB)], osem.at[n])]

    def wait0(nm):
        for cp in copies(nm):
            cp.wait()

    def start0(nm):
        for cp in copies(nm):
            cp.start()

    for nm in STARTS:
        start0(nm)

    wu = [r.bitcast(U32) for r in wb]
    uau = [r.bitcast(U32) for r in ua]
    ubu = [r.bitcast(U32) for r in ub]
    ua_st = [r.at[pl.ds(zero, 5)] for r in ua]
    ub_st = [r.at[pl.ds(zero, 5)] for r in ub]
    pace_st = pace.at[pl.ds(zero, 2)]
    pace[1] = zvec
    for r in uau + ubu:
        r[4, 0:8, :] = zvec
    for r in vb + [va_ref, vb_ref]:
        r.bitcast(U32)[NP, 0, 0:8, :] = zvec

    def params():
        mean, var, g, b = [q[...].astype(F32).reshape(1, C) for q in qs]
        scale = (0.5 * g) * lax.rsqrt(var + 1e-5)
        shift = 0.5 * b - mean * scale
        p_ref[0] = jnp.broadcast_to(0.5 * scale, (8, C))
        p_ref[1] = jnp.broadcast_to(shift, (8, C))
        p_ref[2] = jnp.broadcast_to(0.25 * scale, (8, C))

    def w_chunk(c, r, which, tok):
        sc4 = p_ref[2, 0:1, c * 128:(c + 1) * 128]
        ws = [wu[c][t, r * 8:(r + 1) * 8, :] for t in range(3)]
        if tok is not None:
            ws = [w_ | tok for w_ in ws]
        g0, g1, g2 = [pltpu.bitcast(w_, BF16).astype(F32) * sc4 for w_ in ws]
        gh = 0.5 * g1
        rs = slice(r * 16, (r + 1) * 16)
        if 'a' in which:
            for n, (e, o) in enumerate(((g0 + g2, g1), (0.25 * g2 + g0, gh))):
                ua_st[c][2 * n, rs, :] = (e + o).astype(BF16)
                ua_st[c][2 * n + 1, rs, :] = (e - o).astype(BF16)
        if 'b' in which:
            for n, (e, o) in enumerate(((0.25 * g0 + g2, gh), (g2 - g0, g1))):
                ub_st[c][2 * n, rs, :] = (e + o).astype(BF16)
                ub_st[c][2 * n + 1, rs, :] = (e - o).astype(BF16)

    def rhs_of(c, i):
        if i < 3:
            return wu[c][(2, 0, 1)[i]]
        return uau[c][i - 3] if i < 7 else ubu[c][i - 7]

    def run(segs, xmap, vmap, omap, do_wait, do_start):
        state = {'m': None, 'prod': 0}
        held = {}

        def in_chunk(b, k, tok):
            xr, b0 = xmap(b)
            xs = []
            for j in range(4):
                u = xr[pl.ds(b0 * RU + k * 4 + j, CH, stride=RU), :]
                if tok is not None:
                    u = u | jnp.concatenate([tok] * (CH // 8), axis=0)
                xs += list(_unpack(u))
            v = _in_tf(xs)
            vr, bv = vmap(b)
            vst = vr.at[pl.ds(zero, NP + 1)]
            for i in range(NP):
                vst[i, k, bv:bv + CH, :] = v[i].astype(BF16)

        def side_op(s_, tok):
            if s_ == 'pp':
                params()
            elif s_[0] == 'x':
                in_chunk(s_[1], s_[2], tok)
            else:
                w_chunk(s_[1], s_[2], s_[3], tok)

        def v_token(b):
            return vmap(b)[0].bitcast(U32)[NP, 0, 0:8, :]

        def done_token(todo):
            srcs = {}
            for s_ in todo:
                if s_[0] == 'x':
                    srcs[('x', id(vmap(s_[1])[0]))] = lambda b=s_[1]: v_token(b)
                else:
                    for ch, us in (('a', uau), ('b', ubu)):
                        if ch in s_[3]:
                            srcs[(ch, s_[1])] = lambda r=us[s_[1]]: r[4, 0:8, :]
            tok = None
            for f in srcs.values():
                tok = f() if tok is None else tok | f()
            return tok

        def task(kind, b, c, g, pre, fine, post):
            spans = []
            for bb in range(b, b + g, 32):
                vr, bv = vmap(bb)
                if spans and spans[-1][0] is vr:
                    spans[-1][2] += 32
                else:
                    spans.append([vr, bv, 32])
            spans = [(vr.bitcast(U32), bv, n) for vr, bv, n in spans]
            m = held.pop((b, c), [None] * NP)
            for i in _DOTS[kind]:
                parts = [jnp.concatenate([vru[i, k, bv // 2:(bv + n) // 2, :] for vru, bv, n in spans], axis=0)
                         for k in range(NC)]
                tok = pre()
                if tok is not None:
                    parts[0] = jnp.concatenate([parts[0][0:8] | tok, parts[0][8:]], axis=0)
                for k in range(NC):
                    if fine is not None and state['prod'] % 4 == 0:
                        rows = []
                        for q in range(g // 16):
                            tok = fine()
                            r_ = parts[k][q * 8:(q + 1) * 8]
                            rows.append(r_ if tok is None else r_ | tok)
                        parts[k] = jnp.concatenate(rows, axis=0)
                    state['prod'] += 1
                lhs = pltpu.bitcast(jnp.concatenate(parts, axis=1), BF16)
                m[i] = jnp.dot(lhs, pltpu.bitcast(rhs_of(c, i), BF16), preferred_element_type=F32)
                state['m'] = m[i]
                post()
            if kind in 'ra':
                held[(b, c)] = m
                return
            sc2 = p_ref[0, 0:1, c * 128:(c + 1) * 128]
            sh = p_ref[1, 0:1, c * 128:(c + 1) * 128]
            ys = [h * jnp.tanh(h) + h for h in _out_tf(m, sc2, sh)]
            for j in range(4):
                pk = _pack(ys[2 * j], ys[2 * j + 1])
                for q in range(g // 8):
                    orf, bo = omap(b + q * 8)
                    orf[pl.ds(bo * RU + c * 4 + j, 8, stride=RU), :] = pk[q * 8:(q + 1) * 8]

        def nothing():
            return None

        def segment(main, side, mode):
            npts = sum(len(_DOTS[t[0]]) for t in main)
            st = {'pt': 0, 'done': 0}

            def advance(upto):
                todo = side[st['done']:upto]
                for s_ in todo:
                    side_op(s_, None)
                st['done'] = max(st['done'], upto)
                return done_token(todo)

            if mode == 'D' or (isinstance(mode, tuple) and mode[0] == 'E'):
                if mode == 'D':
                    skip, use = 1, npts
                else:
                    p_, tot = state['prod'], 0
                    for t in main:
                        for _ in range(len(_DOTS[t[0]]) * NC):
                            tot += t[3] // 16 if p_ % 4 == 0 else 0
                            p_ += 1
                    skip, use = mode[1], max(tot - mode[1] - mode[2], 1)

                def point():
                    d = st['pt'] - skip + 1
                    st['pt'] += 1
                    return advance(min(len(side), int(round(len(side) * d / use))) if d > 0 else 0)

                for t in main:
                    if mode == 'D':
                        task(*t, point, None, nothing)
                    else:
                        task(*t, nothing, point, nothing)
                for s_ in side[st['done']:]:
                    side_op(s_, None)
                return

            margin, fake = mode[1:] if isinstance(mode, tuple) else (mode, None)
            last = max(npts - margin, 1)

            def emit():
                upto = min(len(side), -(-(st['pt'] + 1) * len(side) // last))
                todo = side[st['done']:upto]
                for idx, s_ in enumerate(todo):
                    tok = None
                    mi = state['m']
                    if mi is not None:
                        r0 = (idx * (mi.shape[0] // 8) // len(todo)) * 8
                        pace_st[0] = lax.bitcast_convert_type(mi[r0:r0 + 8], U32)
                        tok = pace[1]
                    side_op(s_, tok)
                st['done'] = upto
                st['pt'] += 1

            def pre():
                if fake is not None and st['pt'] == npts:
                    return v_token(fake)
                return None

            emit()
            for t in main:
                task(*t, pre, None, emit)
            assert st['done'] == len(side)

        for waits, starts, main, side, mode in segs:
            if waits:
                for nm in waits:
                    do_wait(nm)
                state['m'] = None
                state['prod'] = 0
            for nm in starts:
                do_start(nm)
            segment(main, side, mode)
        assert not held

    xu = [r.bitcast(U32) for r in xb]
    ou = [r.bitcast(U32) for r in ob]

    def xmap0(b):
        n, b0 = _piece(XP, b)
        return xu[n], b0

    def vmap0(b):
        if b >= BE:
            return va_ref, b - BE
        n, b0 = _piece(VP, b)
        return vb[n], b0

    def omap0(b):
        n, b0 = _piece(OP, b)
        return ou[n], b0

    run(SEGS, xmap0, vmap0, omap0, wait0, start0)
    wait0('l0')

    def body(it, carry):
        r1 = pl.multiple_of(it * (SP * RB), 16)
        r2 = pl.multiple_of(jnp.minimum(it * SP + S2, B - XL0 - S1) * RB, 16)
        x1 = xl.at[pl.ds(r1, S2 * RB)].bitcast(U32)
        x2 = xl.at[pl.ds(r2, S1 * RB)].bitcast(U32)
        lou = [r.at[it].bitcast(U32) for r in lob]

        def mid(_):
            lo_copy(it, 0).start()

            @pl.when(it == 0)
            def _():
                start0('o0')
                start0('o1')
                wait0('l1')

        def xmap(b):
            return (x1, b - S1) if b < SP else (x2, b - SP)

        def vmap(b):
            if b < S1:
                return va_ref, b
            if b < SP:
                return vb_ref, b - S1
            return va_ref, b - SP

        def omap(b):
            n, b0 = _piece(LOP, b)
            return lou[n], b0

        run(LSEGS, xmap, vmap, omap, mid, lambda j: lo_copy(it, j).start())
        for j in range(len(LOP) - 1):
            lo_copy(it, j).wait()
        return carry

    lax.fori_loop(0, NIT, body, 0)

    for n in range(len(OP)):
        wait0('o%d' % n)
    for it in range(NIT):
        lo_copy(it, len(LOP) - 1).wait()


def _compiler_params():
    kw = dict(dimension_semantics=("arbitrary",),
              vmem_limit_bytes=100 * 1024 * 1024,
              disable_bounds_checks=True)
    try:
        return pltpu.CompilerParams(disable_semaphore_checks=True, **kw)
    except TypeError:
        return pltpu.CompilerParams(**kw)


@jax.jit
def pallas_standalone__batchnorm__sampling_kernel(
    x: jax.Array,
    w: jax.Array,
    mean: jax.Array,
    var: jax.Array,
    g: jax.Array,
    b: jax.Array,
):
    assert x.shape == (B, S, C) and w.shape == (3, C, C)
    z = x.reshape(B, S, NC, 128).transpose(0, 2, 1, 3).reshape(B * RB, 128)
    anyspec = pl.BlockSpec(memory_space=pl.ANY)

    def rows(nb):
        return pltpu.VMEM((nb * RB, 128), BF16)

    def vbuf(nb):
        return pltpu.VMEM((NP + 1, NC, nb, 128), BF16)

    scratch = ([rows(b1 - b0) for b0, b1 in XP]
               + [rows(B - XL0)]
               + [vbuf(b1 - b0) for b0, b1 in VP]
               + [vbuf(S1), vbuf(S2)]
               + [rows(b1 - b0) for b0, b1 in OP]
               + [pltpu.VMEM((NIT, (b1 - b0) * RB, 128), BF16) for b0, b1 in LOP]
               + [pltpu.VMEM((3, C, 128), BF16) for _ in range(NC)]
               + [pltpu.VMEM((5, C, 128), BF16) for _ in range(2 * NC)]
               + [pltpu.VMEM((C,), BF16) for _ in range(4)]
               + [pltpu.VMEM((3, 8, C), F32),
                  pltpu.VMEM((2, 8, 128), U32),
                  pltpu.SemaphoreType.DMA((4 + NC + len(XP) + len(LXP),)),
                  pltpu.SemaphoreType.DMA((len(OP) + NIT * len(LOP),))])
    out = pl.pallas_call(
        _kernel,
        grid_spec=pltpu.PrefetchScalarGridSpec(
            num_scalar_prefetch=1,
            grid=(1,),
            in_specs=[anyspec] * 6,
            out_specs=anyspec,
            scratch_shapes=scratch),
        out_shape=jax.ShapeDtypeStruct(z.shape, x.dtype),
        compiler_params=_compiler_params(),
    )(jnp.zeros((1,), jnp.int32), z, w, mean, var, g, b)
    return out.reshape(B, NC, S, 128).transpose(0, 2, 1, 3).reshape(B, S, C)
```
